```python
import jax
import jax.numpy as jnp

def _softmax(x, axis=-1):
    return jax.nn.softmax(x, axis=axis)
def _gelu(x):
    return jax.nn.gelu(x, approximate=True)
def _silu(x):
    return jax.nn.silu(x)
def _sigmoid(x):
    return jax.nn.sigmoid(x)
def _layernorm(x, axis=-1, eps=1e-5):
    m = jnp.mean(x, axis=axis, keepdims=True)
    v = jnp.var(x, axis=axis, keepdims=True)
    return (x - m) / jnp.sqrt(v + eps)
def _scatter_add(tgt, idx, src, axis=0):
    return tgt.at[idx].add(src)
def _segment_sum(src, seg, n):
    return jax.ops.segment_sum(src, seg, n)
class _Rng:
    def __init__(self, key):
        self._k = key
    def _next(self):
        self._k, sub = jax.random.split(self._k)
        return sub
    def normal(self, shape):
        return jax.random.normal(self._next(), shape, dtype=jnp.bfloat16)
    def randint(self, lo, hi, shape):
        return jax.random.randint(self._next(), shape, lo, hi, dtype=jnp.int32)
    def uniform(self, shape, lo=0.0, hi=1.0):
        return jax.random.uniform(self._next(), shape, jnp.bfloat16, lo, hi)
    def permutation(self, n):
        return jax.random.permutation(self._next(), n)


kernel_name = 'standalone__dcn_v2_cross__recsys'

def setup_inputs():
    _rng = _Rng(jax.random.key(int.from_bytes(__import__("os").urandom(4), "little")))
    _w = (lambda a: (lambda t: t.astype(jnp.bfloat16) if jnp.issubdtype(t.dtype, jnp.floating) else t)(jnp.asarray(a)))
    B, F, D, L = 16384, 26, 128, 6
    Din = min(F * D, 1024)
    return {
        "x0": _w((lambda *s: _rng.normal(s) * 0.05)(B, Din)),
        "ws": _w((lambda *s: _rng.normal(s) * 0.05)(L, Din, Din)),
        "bs": _w((lambda *s: _rng.normal(s) * 0.05)(L, Din)),
    }

def reference(x0, ws, bs):
    x = x0
    for l in range(ws.shape[0]):
        x = x0 * (x @ ws[l] + bs[l]) + x
    return x
```

```python
import functools

import jax
import jax.numpy as jnp
import jax.experimental.pallas as pl
import jax.experimental.pallas.tpu as pltpu

_BM = 512


def _kernel(x0_ref, w_ref, b_ref, o_ref, *, n_layers):
    x0 = x0_ref[...].astype(jnp.float32)
    x = x0
    xb = x0_ref[...]
    for l in range(n_layers):
        acc = jnp.dot(xb, w_ref[l], preferred_element_type=jnp.float32)
        x = x0 * (acc + b_ref[l].astype(jnp.float32)) + x
        xb = x.astype(jnp.bfloat16)
    o_ref[...] = xb.astype(o_ref.dtype)


@jax.jit
def pallas_standalone__dcn_v2_cross__recsys_kernel(x0, ws, bs):
    B, D = x0.shape
    L = ws.shape[0]
    bm = _BM
    bs3 = bs.reshape(L, 1, D)
    return pl.pallas_call(
        functools.partial(_kernel, n_layers=L),
        grid=(B // bm,),
        in_specs=[
            pl.BlockSpec((bm, D), lambda i: (i, 0)),
            pl.BlockSpec((L, D, D), lambda i: (0, 0, 0)),
            pl.BlockSpec((L, 1, D), lambda i: (0, 0, 0)),
        ],
        out_specs=pl.BlockSpec((bm, D), lambda i: (i, 0)),
        out_shape=jax.ShapeDtypeStruct((B, D), x0.dtype),
        compiler_params=pltpu.CompilerParams(
            dimension_semantics=("parallel",),
            vmem_limit_bytes=100 * 1024 * 1024,
        ),
    )(x0, ws, bs3)
```

```python
import functools

import numpy as np
import jax
import jax.numpy as jnp
import jax.experimental.pallas as pl
import jax.experimental.pallas.tpu as pltpu

_BM = 512
_LV = 2
_PREP = True

F32 = jnp.float32
BF16 = jnp.bfloat16


def _a_side(q):
    A11, A12, A21, A22 = q
    return [A11 + A22, A21 + A22, A11, A22, A11 + A12, A21 - A11, A12 - A22]


def _b_side(q):
    B11, B12, B21, B22 = q
    return [B11 + B22, B11, B12 - B22, B21 - B11, B22, B11 + B12, B21 + B22]


def _c_side(m):
    M1, M2, M3, M4, M5, M6, M7 = m
    return [M1 + M4 - M5 + M7, M3 + M5, M2 + M4, M1 - M2 + M3 + M6]


class _Blk:
    def __init__(self, g):
        self.g = g

    def __add__(self, o):
        return _Blk([[a + b for a, b in zip(r, s)] for r, s in zip(self.g, o.g)])

    def __sub__(self, o):
        return _Blk([[a - b for a, b in zip(r, s)] for r, s in zip(self.g, o.g)])

    def quads(self):
        h = len(self.g) // 2
        return [_Blk([r[c:c + h] for r in self.g[i:i + h]]) for i in (0, h) for c in (0, h)]


def _leaves(blk, side):
    if len(blk.g) == 1:
        return [blk.g[0][0]]
    return [x for s in side(blk.quads()) for x in _leaves(s, side)]


def _mm(blk, leaf, p=0):
    if len(blk.g) == 1:
        return _Blk([[leaf(blk.g[0][0], p)]])
    m = [_mm(s, leaf, p * 7 + i) for i, s in enumerate(_a_side(blk.quads()))]
    c = _c_side(m)
    return _Blk([a + b for a, b in zip(c[0].g, c[1].g)] + [a + b for a, b in zip(c[2].g, c[3].g)])


def _kernel(x0_ref, w_ref, b_ref, o_ref, t_ref, *, n_layers):
    n = 2 ** _LV
    D = x0_ref.shape[1]
    H = D // n
    h = x0_ref.shape[0] // n
    cs = [slice(i * H, (i + 1) * H) for i in range(n)]
    rs = [slice(i * h, (i + 1) * h) for i in range(n)]

    if _PREP:
        @pl.when(pl.program_id(0) == 0)
        def _():
            def body(l, c):
                Bm = _Blk([[w_ref[l, r, cc].astype(F32) for cc in cs] for r in cs])
                for p, t in enumerate(_leaves(Bm, _b_side)):
                    t_ref[l, p] = t.astype(BF16)
                return c
            jax.lax.fori_loop(0, n_layers, body, 0)

    X = [[x0_ref[r, c].astype(F32) for c in cs] for r in rs]
    A = X
    for l in range(n_layers):
        bb = [b_ref[l:l + 1, c].astype(F32) for c in cs]
        C = _mm(_Blk(A), lambda a, p: jnp.dot(a.astype(BF16), t_ref[l, p], preferred_element_type=F32)).g
        A = [[X[i][j] * (C[i][j] + bb[j]) + A[i][j] for j in range(n)] for i in range(n)]
    for i in range(n):
        for j in range(n):
            o_ref[rs[i], cs[j]] = A[i][j].astype(o_ref.dtype)


@jax.jit
def pallas_standalone__dcn_v2_cross__recsys_kernel(x0, ws, bs):
    B, D = x0.shape
    L = ws.shape[0]
    bm = _BM
    return pl.pallas_call(
        functools.partial(_kernel, n_layers=L),
        grid=(B // bm,),
        in_specs=[
            pl.BlockSpec((bm, D), lambda i: (i, 0)),
            pl.BlockSpec((L, D, D), lambda i: (0, 0, 0)),
            pl.BlockSpec((L, D), lambda i: (0, 0)),
        ],
        out_specs=pl.BlockSpec((bm, D), lambda i: (i, 0)),
        out_shape=jax.ShapeDtypeStruct((B, D), x0.dtype),
        scratch_shapes=[pltpu.VMEM((L, 7 ** _LV, D >> _LV, D >> _LV), BF16)],
        compiler_params=pltpu.CompilerParams(
            dimension_semantics=("arbitrary",),
            vmem_limit_bytes=120 * 1024 * 1024,
        ),
    )(x0, ws, bs)
```

```python
import functools

import numpy as np
import jax
import jax.numpy as jnp
import jax.experimental.pallas as pl
import jax.experimental.pallas.tpu as pltpu

_BM = 512
_LV = 2

F32 = jnp.float32
BF16 = jnp.bfloat16


def _a_side(q):
    A11, A12, A21, A22 = q
    return [A11 + A22, A21 + A22, A11, A22, A11 + A12, A21 - A11, A12 - A22]


def _b_side(q):
    B11, B12, B21, B22 = q
    return [B11 + B22, B11, B12 - B22, B21 - B11, B22, B11 + B12, B21 + B22]


def _c_side(m):
    M1, M2, M3, M4, M5, M6, M7 = m
    return [M1 + M4 - M5 + M7, M3 + M5, M2 + M4, M1 - M2 + M3 + M6]


class _Blk:
    def __init__(self, g):
        self.g = g

    def __add__(self, o):
        return _Blk([[a + b for a, b in zip(r, s)] for r, s in zip(self.g, o.g)])

    def __sub__(self, o):
        return _Blk([[a - b for a, b in zip(r, s)] for r, s in zip(self.g, o.g)])

    def quads(self):
        h = len(self.g) // 2
        return [_Blk([r[c:c + h] for r in self.g[i:i + h]]) for i in (0, h) for c in (0, h)]


def _leaves(blk, side):
    if len(blk.g) == 1:
        return [blk.g[0][0]]
    return [x for s in side(blk.quads()) for x in _leaves(s, side)]


def _mm(blk, leaf, p=0):
    if len(blk.g) == 1:
        return _Blk([[leaf(blk.g[0][0], p)]])
    m = [_mm(s, leaf, p * 7 + i) for i, s in enumerate(_a_side(blk.quads()))]
    c = _c_side(m)
    return _Blk([a + b for a, b in zip(c[0].g, c[1].g)] + [a + b for a, b in zip(c[2].g, c[3].g)])


def _kernel(x0_ref, w_hbm, b_ref, o_ref, t_ref, w_ref, sem, *, n_layers):
    n = 2 ** _LV
    D = x0_ref.shape[1]
    H = D // n
    h = x0_ref.shape[0] // n
    cs = [slice(i * H, (i + 1) * H) for i in range(n)]
    rs = [slice(i * h, (i + 1) * h) for i in range(n)]

    if True:
        @pl.when(pl.program_id(0) == 0)
        def _():
            def dma(l):
                return pltpu.make_async_copy(w_hbm.at[l], w_ref.at[l], sem.at[l])

            for l in range(n_layers):
                dma(l).start()

            def body(l, c):
                dma(l).wait()
                Bm = _Blk([[w_ref[l, r, cc].astype(F32) for cc in cs] for r in cs])
                for p, t in enumerate(_leaves(Bm, _b_side)):
                    t_ref[l, p] = pltpu.bitcast(t.astype(BF16), jnp.uint32)
                return c
            jax.lax.fori_loop(0, n_layers, body, 0)

    X = [[x0_ref[r, c].astype(F32) for c in cs] for r in rs]
    A = X
    for l in range(n_layers):
        bb = [b_ref[l:l + 1, c].astype(F32) for c in cs]
        C = _mm(_Blk(A), lambda a, p: jnp.dot(a.astype(BF16), pltpu.bitcast(t_ref[l, p], BF16), preferred_element_type=F32)).g
        A = [[X[i][j] * (C[i][j] + bb[j]) + A[i][j] for j in range(n)] for i in range(n)]
    for i in range(n):
        for j in range(n):
            o_ref[rs[i], cs[j]] = A[i][j].astype(o_ref.dtype)


@jax.jit
def pallas_standalone__dcn_v2_cross__recsys_kernel(x0, ws, bs):
    B, D = x0.shape
    L = ws.shape[0]
    bm = _BM
    return pl.pallas_call(
        functools.partial(_kernel, n_layers=L),
        grid=(B // bm,),
        in_specs=[
            pl.BlockSpec((bm, D), lambda i: (i, 0)),
            pl.BlockSpec(memory_space=pl.ANY),
            pl.BlockSpec((L, D), lambda i: (0, 0)),
        ],
        out_specs=pl.BlockSpec((bm, D), lambda i: (i, 0)),
        out_shape=jax.ShapeDtypeStruct((B, D), x0.dtype),
        scratch_shapes=[pltpu.VMEM((L, 7 ** _LV, D >> _LV + 1, D >> _LV), jnp.uint32),
                        pltpu.VMEM((L, D, D), BF16), pltpu.SemaphoreType.DMA((L,))],
        compiler_params=pltpu.CompilerParams(
            dimension_semantics=("arbitrary",),
            vmem_limit_bytes=120 * 1024 * 1024,
        ),
    )(x0, ws, bs)
```
